```python
import os as _os
_os.environ.setdefault("JAX_PLATFORMS", "cpu")
import jax
import jax.numpy as jnp

def _softmax(x, axis=-1):
    return jax.nn.softmax(x, axis=axis)
def _gelu(x):
    return jax.nn.gelu(x, approximate=True)
def _silu(x):
    return jax.nn.silu(x)
def _sigmoid(x):
    return jax.nn.sigmoid(x)
def _layernorm(x, axis=-1, eps=1e-5):
    m = jnp.mean(x, axis=axis, keepdims=True)
    v = jnp.var(x, axis=axis, keepdims=True)
    return (x - m) / jnp.sqrt(v + eps)
def _scatter_add(tgt, idx, src, axis=0):
    return tgt.at[idx].add(src)
def _segment_sum(src, seg, n):
    return jax.ops.segment_sum(src, seg, n)
class _Rng:
    def __init__(self, key):
        self._k = key
    def _next(self):
        self._k, sub = jax.random.split(self._k)
        return sub
    def normal(self, shape):
        return jax.random.normal(self._next(), shape, dtype=jnp.bfloat16)
    def randint(self, lo, hi, shape):
        return jax.random.randint(self._next(), shape, lo, hi, dtype=jnp.int32)
    def uniform(self, shape, lo=0.0, hi=1.0):
        return jax.random.uniform(self._next(), shape, jnp.bfloat16, lo, hi)
    def permutation(self, n):
        return jax.random.permutation(self._next(), n)


kernel_name = 'gated_mix__mha_block__softmax_full_mha__prompt'

def setup_inputs():
    _rng = _Rng(jax.random.key(int.from_bytes(__import__("os").urandom(4), "little")))
    _w = (lambda a: (lambda t: t.astype(jnp.bfloat16) if jnp.issubdtype(t.dtype, jnp.floating) else t)(jnp.asarray(a)))
    def _A_setup():
        B, S, D, H = 1, 2048, 448, 16
        return {
            "x": _w((lambda *s: _rng.normal(s) * 0.05)(B, S, D)),
            "wqkv": _w((lambda *s: _rng.normal(s) * 0.4)(D, 3 * D)),
            "wo": _w((lambda *s: _rng.normal(s) * 0.05)(D, D)),
        }
    _A_in = _A_setup()

    def _B_setup():
        B, S, D = 1, 2048, 448
        return {
            "x": _w((lambda *s: _rng.normal(s) * 0.05)(B, S, D)),
            "wqkv": _w((lambda *s: _rng.normal(s) * 0.4)(D, 3 * D)),
            "wo": _w((lambda *s: _rng.normal(s) * 0.05)(D, D)),
        }
    _B_in = _B_setup()

    return {
        "A_x": _A_in["x"],
        "A_wqkv": _A_in["wqkv"],
        "A_wo": _A_in["wo"],
        "B_x": _B_in["x"],
        "B_wqkv": _B_in["wqkv"],
        "B_wo": _B_in["wo"],
        "gate_w": _w((lambda *s: _rng.normal(s) * 0.05)(448) * 16.0),
    }

def reference(A_x, A_wqkv, A_wo, B_x, B_wqkv, B_wo, gate_w):
    def _A_ref(x, wqkv, wo):
        B, S, D = x.shape
        H = 16
        Dh = D // H
        qkv = (lambda x, *d: x.transpose(*d))((x @ wqkv).reshape(B, S, 3, H, Dh), 2, 0, 3, 1, 4)
        q, k, v = qkv[0], qkv[1], qkv[2]
        scores = jnp.einsum("bhqd,bhkd->bhqk", q, k) * (Dh ** -0.5)
        p = _softmax(scores, axis=-1)
        o = jnp.einsum("bhqk,bhkd->bhqd", p, v)
        return (lambda x, *d: x.transpose(*d))(o, 0, 2, 1, 3).reshape(B, S, D) @ wo

    def _B_ref(x, wqkv, wo):
        B, S, D = x.shape
        H = 16; Dh = D // H
        qkv = (lambda x, *d: x.transpose(*d))((x @ wqkv).reshape(B, S, 3, H, Dh), 2, 0, 3, 1, 4)
        q, k, v = qkv[0], qkv[1], qkv[2]
        scale = Dh ** -0.5
        scores = jnp.einsum("bhqd,bhkd->bhqk", q, k) * scale
        p = _softmax(scores, axis=-1)
        o = jnp.einsum("bhqk,bhkd->bhqd", p, v)
        return (lambda x, *d: x.transpose(*d))(o, 0, 2, 1, 3).reshape(B, S, D) @ wo

    x = A_x
    g = _sigmoid((x * gate_w).sum(-1, keepdims=True))
    a = _A_ref(x, A_wqkv, A_wo)
    b = _B_ref(x, B_wqkv, B_wo)
    return g * a + (1 - g) * b
```

```python
import math
import jax
import jax.numpy as jnp
from jax import lax
import jax.experimental.pallas as pl
import jax.experimental.pallas.tpu as pltpu

S = 2048; D = 448; H = 16; DH = 28; HP = 32
NG = 8
NH = 32
GW = 128
NP = NH * HP
BQ = 512
KC = 128
UN = 6
CH = 512
NC = S // KC
QSCALE = (DH ** -0.5) * math.log2(math.e)
F32 = jnp.float32
BF16 = jnp.bfloat16


def _kernel(xt_ref, xtq_ref, wa_ref, wb_ref, woa_ref, wob_ref, gw_ref, o_ref,
            wt_s, wop_s, wot_s, ktp_s, k_s, vt_s, qt_s, ot_s, sa_s, sb_s):
    i = pl.program_id(0)

    def scatter_heads(dst, b, val, cols):
        for h in range(H):
            r0 = (b * H + h) * HP
            dst[r0:r0 + DH, cols] = val[h * DH:(h + 1) * DH, :].astype(dst.dtype)

    @pl.when(i == 0)
    def _():
        for b, w_ref in enumerate((wa_ref, wb_ref)):
            wt_s[b] = w_ref[...].astype(F32).T.astype(BF16)
        wop_s[...] = jnp.zeros(wop_s.shape, F32)
        for b, wo_ref in enumerate((woa_ref, wob_ref)):
            scatter_heads(wop_s, b, wo_ref[...].astype(F32), slice(None))
        wot_s[...] = wop_s[...].T.astype(BF16)
        ktp_s[...] = jnp.zeros(ktp_s.shape, F32)
        qt_s[...] = jnp.zeros(qt_s.shape, BF16)
        rowi = lax.broadcasted_iota(jnp.int32, vt_s.shape, 0)
        vt_s[...] = jnp.where(rowi % HP == DH, 1.0, 0.0).astype(BF16)

        def kv_body(c, carry):
            c0 = pl.multiple_of(c * CH, CH)
            xc = xt_ref[:, pl.ds(c0, CH)]
            for b in range(2):
                kt = jnp.dot(wt_s[b, D:2 * D, :], xc, preferred_element_type=F32)
                scatter_heads(ktp_s, b, kt, slice(None))
                vt = jnp.dot(wt_s[b, 2 * D:3 * D, :], xc, preferred_element_type=F32)
                scatter_heads(vt_s, b, vt, pl.ds(c0, CH))
            k_s[pl.ds(c0, CH), :] = ktp_s[...].T.astype(BF16)
            return carry
        lax.fori_loop(0, S // CH, kv_body, 0)

    xq = xtq_ref[...]
    for b in range(2):
        qt = jnp.dot(wt_s[b, 0:D, :], xq, preferred_element_type=F32) * QSCALE
        scatter_heads(qt_s, b, qt, slice(None))

    row = lax.broadcasted_iota(jnp.int32, (GW, BQ), 0)

    def masked_q(h):
        goff = pl.multiple_of((h // 4) * GW, GW)
        qtg = qt_s[pl.ds(goff, GW), :]
        return goff, jnp.where((row // HP) == (h % 4), qtg, jnp.zeros_like(qtg))

    def s1_chunk(c, goff, qm, s_ref, m8):
        st = jnp.dot(k_s[c * KC:(c + 1) * KC, pl.ds(goff, GW)], qm, preferred_element_type=F32)
        s_ref[c * KC:(c + 1) * KC, :] = st
        cm = jnp.max(st.reshape(KC // 8, 8, BQ), axis=0)
        return cm if m8 is None else jnp.maximum(m8, cm)

    def s2_chunk(c, hoff, s_ref, m, acc):
        pt = jnp.exp2(s_ref[c * KC:(c + 1) * KC, :] - m).astype(BF16)
        o = jnp.dot(vt_s[pl.ds(hoff, HP), c * KC:(c + 1) * KC], pt, preferred_element_type=F32)
        return o if acc is None else acc + o

    def fused(h1, s1_ref, h2, s2_ref, m2):
        goff, qm = masked_q(h1)
        hoff = pl.multiple_of(h2 * HP, HP)
        m8 = None; acc = None
        for c in range(NC):
            m8 = s1_chunk(c, goff, qm, s1_ref, m8)
            acc = s2_chunk(c, hoff, s2_ref, m2, acc)
        ot_s[pl.ds(hoff, HP), :] = (acc * (1.0 / acc[DH:DH + 1, :])).astype(BF16)
        return jnp.max(m8, axis=0, keepdims=True)

    goff, qm = masked_q(0)
    m8 = None
    for c in range(NC):
        m8 = s1_chunk(c, goff, qm, sa_s, m8)
    ma = jnp.max(m8, axis=0, keepdims=True)

    def pair(h, ma):
        mb = fused(h + 1, sb_s, h, sa_s, ma)
        return fused(h + 2, sa_s, h + 1, sb_s, mb)

    def body(j, ma):
        for u in range(UN // 2):
            ma = pair(UN * j + 2 * u, ma)
        return ma

    nit = (NH - 2) // UN
    ma = lax.fori_loop(0, nit, body, ma)
    for h in range(nit * UN, NH - 2, 2):
        ma = pair(h, ma)
    mb = fused(NH - 1, sb_s, NH - 2, sa_s, ma)
    hoff = (NH - 1) * HP
    acc = None
    for c in range(NC):
        acc = s2_chunk(c, hoff, sb_s, mb, acc)
    ot_s[hoff:hoff + HP, :] = (acc * (1.0 / acc[DH:DH + 1, :])).astype(BF16)

    a = jnp.dot(wot_s[:, :512], ot_s[:512, :], preferred_element_type=F32)
    b = jnp.dot(wot_s[:, 512:], ot_s[512:, :], preferred_element_type=F32)
    gl = jnp.dot(gw_ref[...], xq, preferred_element_type=F32)[0:1, :]
    gt = jax.nn.sigmoid(gl)
    o_ref[...] = (gt * a + (1.0 - gt) * b).astype(o_ref.dtype)


@jax.jit
def pallas_gated_mix__mha_block__softmax_full_mha__prompt_kernel(A_x, A_wqkv, A_wo, B_x, B_wqkv, B_wo, gate_w):
    xt = A_x.reshape(S, D).T
    gw = jnp.broadcast_to(gate_w.reshape(1, D), (8, D))
    full = lambda shp: pl.BlockSpec(shp, lambda i: (0,) * len(shp))
    out = pl.pallas_call(
        _kernel,
        grid=(S // BQ,),
        in_specs=[full((D, S)), pl.BlockSpec((D, BQ), lambda i: (0, i)),
                  full((D, 3 * D)), full((D, 3 * D)), full((D, D)), full((D, D)), full((8, D))],
        out_specs=pl.BlockSpec((D, BQ), lambda i: (0, i)),
        out_shape=jax.ShapeDtypeStruct((D, S), BF16),
        scratch_shapes=[pltpu.VMEM((2, 3 * D, D), BF16),
                        pltpu.VMEM((NP, D), F32),
                        pltpu.VMEM((D, NP), BF16),
                        pltpu.VMEM((NP, CH), F32),
                        pltpu.VMEM((S, NP), BF16),
                        pltpu.VMEM((NP, S), BF16),
                        pltpu.VMEM((NP, BQ), BF16),
                        pltpu.VMEM((NP, BQ), BF16),
                        pltpu.VMEM((S, BQ), F32),
                        pltpu.VMEM((S, BQ), F32)],
        compiler_params=pltpu.CompilerParams(dimension_semantics=("arbitrary",),
                                             vmem_limit_bytes=100 * 1024 * 1024),
    )(xt, xt, A_wqkv, B_wqkv, A_wo, B_wo, gw)
    return out.T.reshape(1, S, D)
```

```python
import math
import jax
import jax.numpy as jnp
from jax import lax
import jax.experimental.pallas as pl
import jax.experimental.pallas.tpu as pltpu

S = 2048; D = 448; H = 16; DH = 28; HP = 32
NH = 32
GW = 128
NP = NH * HP
BQ = 512
NQ = S // BQ
NT = NQ * NH
KC = 128
UN = 6
CH = 512
NC = S // KC
QSCALE = (DH ** -0.5) * math.log2(math.e)
F32 = jnp.float32
BF16 = jnp.bfloat16


def _kernel(xt_hbm, wa_hbm, wb_hbm, woa_hbm, wob_hbm, gw_ref, o_hbm,
            xt_s, w_s, wo_s, wt_s, wop_s, wot_s, ktp_s, k_s, vt_s, qt_s, ot_s, sa_s, sb_s, ob_s,
            sem_w, sem_x, sem_o):
    w_cp = [pltpu.make_async_copy(src, w_s.at[b], sem_w.at[b]) for b, src in enumerate((wa_hbm, wb_hbm))]
    wo_cp = [pltpu.make_async_copy(src, wo_s.at[b], sem_w.at[2 + b]) for b, src in enumerate((woa_hbm, wob_hbm))]
    x_cp = [pltpu.make_async_copy(xt_hbm.at[:, c * CH:(c + 1) * CH], xt_s.at[:, c * CH:(c + 1) * CH], sem_x.at[c])
            for c in range(S // CH)]
    w_cp[0].start(); w_cp[1].start(); x_cp[0].start()
    wo_cp[0].start(); wo_cp[1].start()
    for cp in x_cp[1:]:
        cp.start()

    def scatter_heads(dst, b, val, cols):
        for h in range(H):
            r0 = (b * H + h) * HP
            dst[r0:r0 + DH, cols] = val[h * DH:(h + 1) * DH, :].astype(dst.dtype)

    ktp_s[...] = jnp.zeros(ktp_s.shape, F32)
    qt_s[...] = jnp.zeros(qt_s.shape, BF16)
    wop_s[...] = jnp.zeros(wop_s.shape, F32)
    rowi = lax.broadcasted_iota(jnp.int32, vt_s.shape, 0)
    vt_s[...] = jnp.where(rowi % HP == DH, 1.0, 0.0).astype(BF16)
    for b in range(2):
        w_cp[b].wait()
        wt_s[b] = w_s[b].astype(F32).T.astype(BF16)
    for b in range(2):
        wo_cp[b].wait()
        scatter_heads(wop_s, b, wo_s[b].astype(F32), slice(None))
    wot_s[...] = wop_s[...].T.astype(BF16)
    for cp in x_cp:
        cp.wait()

    def kv_body(c, carry):
        c0 = pl.multiple_of(c * CH, CH)
        xc = xt_s[:, pl.ds(c0, CH)]
        for b in range(2):
            kt = jnp.dot(wt_s[b, D:2 * D, :], xc, preferred_element_type=F32)
            scatter_heads(ktp_s, b, kt, slice(None))
            vt = jnp.dot(wt_s[b, 2 * D:3 * D, :], xc, preferred_element_type=F32)
            scatter_heads(vt_s, b, vt, pl.ds(c0, CH))
            qt = jnp.dot(wt_s[b, 0:D, :], xc, preferred_element_type=F32) * QSCALE
            scatter_heads(qt_s, b, qt, pl.ds(c0, CH))
        k_s[pl.ds(c0, CH), :] = ktp_s[...].T.astype(BF16)
        return carry
    lax.fori_loop(0, S // CH, kv_body, 0)

    row = lax.broadcasted_iota(jnp.int32, (GW, BQ), 0)

    def aligned(v, m):
        return v if isinstance(v, int) else pl.multiple_of(v, m)

    def masked_q(t):
        h = t % NH
        goff = aligned((h // 4) * GW, GW)
        qoff = aligned((t // NH) * BQ, BQ)
        qtg = qt_s[pl.ds(goff, GW), pl.ds(qoff, BQ)]
        return goff, jnp.where((row // HP) == (h % 4), qtg, jnp.zeros_like(qtg))

    def s1_chunk(c, goff, qm, s_ref, m8):
        st = jnp.dot(k_s[c * KC:(c + 1) * KC, pl.ds(goff, GW)], qm, preferred_element_type=F32)
        s_ref[c * KC:(c + 1) * KC, :] = st
        cm = jnp.max(st.reshape(KC // 8, 8, BQ), axis=0)
        return cm if m8 is None else jnp.maximum(m8, cm)

    def s2_chunk(c, hoff, s_ref, m, acc):
        pt = jnp.exp2(s_ref[c * KC:(c + 1) * KC, :] - m).astype(BF16)
        o = jnp.dot(vt_s[pl.ds(hoff, HP), c * KC:(c + 1) * KC], pt, preferred_element_type=F32)
        return o if acc is None else acc + o

    def stages(t1, s1_ref, t2, s2_ref, m2):
        if t1 is not None:
            goff, qm = masked_q(t1)
        if t2 is not None:
            hoff = aligned((t2 % NH) * HP, HP)
            qoff = aligned((t2 // NH) * BQ, BQ)
        m8 = None; acc = None
        for c in range(NC):
            if t1 is not None:
                m8 = s1_chunk(c, goff, qm, s1_ref, m8)
            if t2 is not None:
                acc = s2_chunk(c, hoff, s2_ref, m2, acc)
        if t2 is not None:
            ot_s[pl.ds(hoff, HP), pl.ds(qoff, BQ)] = (acc * (1.0 / acc[DH:DH + 1, :])).astype(BF16)
        if t1 is not None:
            return jnp.max(m8, axis=0, keepdims=True)

    ma = stages(0, sa_s, None, None, None)

    def pair(t, ma):
        mb = stages(t + 1, sb_s, t, sa_s, ma)
        return stages(t + 2, sa_s, t + 1, sb_s, mb)

    def body(j, ma):
        for u in range(UN // 2):
            ma = pair(UN * j + 2 * u, ma)
        return ma

    nit = (NT - 2) // UN
    ma = lax.fori_loop(0, nit, body, ma)
    for t in range(nit * UN, NT - 2, 2):
        ma = pair(t, ma)
    mb = stages(NT - 1, sb_s, NT - 2, sa_s, ma)
    stages(None, None, NT - 1, sb_s, mb)

    o_cp = []
    for c in range(NQ):
        cs = slice(c * BQ, (c + 1) * BQ)
        a = jnp.dot(wot_s[:, :512], ot_s[:512, cs], preferred_element_type=F32)
        b = jnp.dot(wot_s[:, 512:], ot_s[512:, cs], preferred_element_type=F32)
        gl = jnp.dot(gw_ref[...], xt_s[:, cs], preferred_element_type=F32)[0:1, :]
        gt = jax.nn.sigmoid(gl)
        ob_s[:, cs] = (gt * a + (1.0 - gt) * b).astype(BF16)
        cp = pltpu.make_async_copy(ob_s.at[:, cs], o_hbm.at[:, cs], sem_o.at[c])
        cp.start()
        o_cp.append(cp)
    for cp in o_cp:
        cp.wait()


@jax.jit
def pallas_gated_mix__mha_block__softmax_full_mha__prompt_kernel(A_x, A_wqkv, A_wo, B_x, B_wqkv, B_wo, gate_w):
    xt = A_x.reshape(S, D).T
    gw = jnp.broadcast_to(gate_w.reshape(1, D), (8, D))
    hbm = pl.BlockSpec(memory_space=pl.ANY)
    out = pl.pallas_call(
        _kernel,
        in_specs=[hbm, hbm, hbm, hbm, hbm, pl.BlockSpec(memory_space=pltpu.VMEM)],
        out_specs=hbm,
        out_shape=jax.ShapeDtypeStruct((D, S), BF16),
        scratch_shapes=[pltpu.VMEM((D, S), BF16),
                        pltpu.VMEM((2, D, 3 * D), BF16),
                        pltpu.VMEM((2, D, D), BF16),
                        pltpu.VMEM((2, 3 * D, D), BF16),
                        pltpu.VMEM((NP, D), F32),
                        pltpu.VMEM((D, NP), BF16),
                        pltpu.VMEM((NP, CH), F32),
                        pltpu.VMEM((S, NP), BF16),
                        pltpu.VMEM((NP, S), BF16),
                        pltpu.VMEM((NP, S), BF16),
                        pltpu.VMEM((NP, S), BF16),
                        pltpu.VMEM((S, BQ), F32),
                        pltpu.VMEM((S, BQ), F32),
                        pltpu.VMEM((D, S), BF16),
                        pltpu.SemaphoreType.DMA((4,)),
                        pltpu.SemaphoreType.DMA((S // CH,)),
                        pltpu.SemaphoreType.DMA((NQ,))],
        compiler_params=pltpu.CompilerParams(vmem_limit_bytes=100 * 1024 * 1024),
    )(xt, A_wqkv, B_wqkv, A_wo, B_wo, gw)
    return out.T.reshape(1, S, D)
```

```python
import math

import jax
import jax.numpy as jnp
from jax import lax
import jax.experimental.pallas as pl
import jax.experimental.pallas.tpu as pltpu

S = 2048
D = 448
H = 16
DH = 28
HP = 32
NH = 2 * H
GW = 128
NP = NH * HP
BQ = 512
NQ = S // BQ
NT = NQ * NH
KC = 128
NC = S // KC
UN = 6
CH = 512
QSCALE = (DH ** -0.5) * math.log2(math.e)
F32 = jnp.float32
BF16 = jnp.bfloat16


def _aligned(v, m):
    return v if isinstance(v, int) else pl.multiple_of(v, m)


def _kernel(xt_hbm, wa_hbm, wb_hbm, woa_hbm, wob_hbm, gw_ref, o_hbm,
            xt_s, w_s, wo_s, wt_s, wop_s, wot_s, ktp_s, k_s, vt_s, qt_s, ot_s, sa_s, sb_s, ob_s,
            sem_w, sem_x, sem_o):
    w_cp = [pltpu.make_async_copy(src, w_s.at[b], sem_w.at[b])
            for b, src in enumerate((wa_hbm, wb_hbm))]
    wo_cp = [pltpu.make_async_copy(src, wo_s.at[b], sem_w.at[2 + b])
             for b, src in enumerate((woa_hbm, wob_hbm))]

    def x_cp(c):
        c0 = _aligned(c * CH, CH)
        return pltpu.make_async_copy(xt_hbm.at[:, pl.ds(c0, CH)], xt_s.at[:, pl.ds(c0, CH)],
                                     sem_x.at[c])

    for cp in w_cp:
        cp.start()
    for c in range(S // CH):
        x_cp(c).start()
    for cp in wo_cp:
        cp.start()

    def scatter_heads(dst, b, val, cols):
        for h in range(H):
            r0 = (b * H + h) * HP
            dst[r0:r0 + DH, cols] = val[h * DH:(h + 1) * DH, :].astype(dst.dtype)

    ktp_s[...] = jnp.zeros(ktp_s.shape, F32)
    qt_s[...] = jnp.zeros(qt_s.shape, BF16)
    rowi = lax.broadcasted_iota(jnp.int32, vt_s.shape, 0)
    vt_s[...] = jnp.where(rowi % HP == DH, 1.0, 0.0).astype(BF16)
    for b in range(2):
        w_cp[b].wait()
        wt_s[b] = w_s[b].astype(F32).T.astype(BF16)

    def proj_body(c, carry):
        c0 = pl.multiple_of(c * CH, CH)
        x_cp(c).wait()
        xc = xt_s[:, pl.ds(c0, CH)]
        for b in range(2):
            kt = jnp.dot(wt_s[b, D:2 * D, :], xc, preferred_element_type=F32)
            scatter_heads(ktp_s, b, kt, slice(None))
            vt = jnp.dot(wt_s[b, 2 * D:3 * D, :], xc, preferred_element_type=F32)
            scatter_heads(vt_s, b, vt, pl.ds(c0, CH))
            qt = jnp.dot(wt_s[b, 0:D, :], xc, preferred_element_type=F32) * QSCALE
            scatter_heads(qt_s, b, qt, pl.ds(c0, CH))
        k_s[pl.ds(c0, CH), :] = ktp_s[...].T.astype(BF16)
        return carry

    lax.fori_loop(0, S // CH, proj_body, 0)

    row = lax.broadcasted_iota(jnp.int32, (GW, BQ), 0)

    def stages(t1, s1_ref, t2, s2_ref, m2):
        if t1 is not None:
            h1 = t1 % NH
            goff = _aligned((h1 // 4) * GW, GW)
            qtg = qt_s[pl.ds(goff, GW), pl.ds(_aligned((t1 // NH) * BQ, BQ), BQ)]
            qm = jnp.where((row // HP) == (h1 % 4), qtg, jnp.zeros_like(qtg))
        if t2 is not None:
            hoff = _aligned((t2 % NH) * HP, HP)
            qoff = _aligned((t2 // NH) * BQ, BQ)
        m8 = None
        acc = None
        for c in range(NC):
            ks = slice(c * KC, (c + 1) * KC)
            if t1 is not None:
                st = jnp.dot(k_s[ks, pl.ds(goff, GW)], qm, preferred_element_type=F32)
                s1_ref[ks, :] = st
                cm = jnp.max(st.reshape(KC // 8, 8, BQ), axis=0)
                m8 = cm if m8 is None else jnp.maximum(m8, cm)
            if t2 is not None:
                pt = jnp.exp2(s2_ref[ks, :] - m2).astype(BF16)
                o = jnp.dot(vt_s[pl.ds(hoff, HP), ks], pt, preferred_element_type=F32)
                acc = o if acc is None else acc + o
        if t2 is not None:
            ot_s[pl.ds(hoff, HP), pl.ds(qoff, BQ)] = (
                acc * (1.0 / acc[DH:DH + 1, :])).astype(BF16)
        if t1 is not None:
            return jnp.max(m8, axis=0, keepdims=True)
        return None

    def loop_body(j, ma):
        for u in range(0, UN, 2):
            t = UN * j + u
            mb = stages(t + 1, sb_s, t, sa_s, ma)
            ma = stages(t + 2, sa_s, t + 1, sb_s, mb)
        return ma

    ma = stages(0, sa_s, None, None, None)
    ma = lax.fori_loop(0, (NT - 2) // UN, loop_body, ma)

    wop_s[...] = jnp.zeros(wop_s.shape, F32)
    for b in range(2):
        wo_cp[b].wait()
        scatter_heads(wop_s, b, wo_s[b].astype(F32), slice(None))
    wot_s[...] = wop_s[...].T.astype(BF16)

    mb = stages(NT - 1, sb_s, NT - 2, sa_s, ma)
    stages(None, None, NT - 1, sb_s, mb)

    o_cp = []
    half = NP // 2
    for c in range(NQ):
        cs = slice(c * BQ, (c + 1) * BQ)
        a = jnp.dot(wot_s[:, :half], ot_s[:half, cs], preferred_element_type=F32)
        b = jnp.dot(wot_s[:, half:], ot_s[half:, cs], preferred_element_type=F32)
        gl = jnp.dot(gw_ref[...], xt_s[:, cs], preferred_element_type=F32)[0:1, :]
        gt = jax.nn.sigmoid(gl)
        ob_s[:, cs] = (gt * a + (1.0 - gt) * b).astype(BF16)
        cp = pltpu.make_async_copy(ob_s.at[:, cs], o_hbm.at[:, cs], sem_o.at[c])
        cp.start()
        o_cp.append(cp)
    for cp in o_cp:
        cp.wait()


@jax.jit
def pallas_gated_mix__mha_block__softmax_full_mha__prompt_kernel(
    A_x: jax.Array,
    A_wqkv: jax.Array,
    A_wo: jax.Array,
    B_x: jax.Array,
    B_wqkv: jax.Array,
    B_wo: jax.Array,
    gate_w: jax.Array,
):
    del B_x
    assert (NT - 2) % UN == 0 and UN % 2 == 0
    xt = A_x.reshape(S, D).T
    gw = jnp.broadcast_to(gate_w.reshape(1, D), (8, D))
    hbm = pl.BlockSpec(memory_space=pl.ANY)
    out_t = pl.pallas_call(
        _kernel,
        in_specs=[hbm, hbm, hbm, hbm, hbm, pl.BlockSpec(memory_space=pltpu.VMEM)],
        out_specs=hbm,
        out_shape=jax.ShapeDtypeStruct((D, S), BF16),
        scratch_shapes=[
            pltpu.VMEM((D, S), BF16),
            pltpu.VMEM((2, D, 3 * D), BF16),
            pltpu.VMEM((2, D, D), BF16),
            pltpu.VMEM((2, 3 * D, D), BF16),
            pltpu.VMEM((NP, D), F32),
            pltpu.VMEM((D, NP), BF16),
            pltpu.VMEM((NP, CH), F32),
            pltpu.VMEM((S, NP), BF16),
            pltpu.VMEM((NP, S), BF16),
            pltpu.VMEM((NP, S), BF16),
            pltpu.VMEM((NP, S), BF16),
            pltpu.VMEM((S, BQ), F32),
            pltpu.VMEM((S, BQ), F32),
            pltpu.VMEM((D, S), BF16),
            pltpu.SemaphoreType.DMA((4,)),
            pltpu.SemaphoreType.DMA((S // CH,)),
            pltpu.SemaphoreType.DMA((NQ,)),
        ],
        compiler_params=pltpu.CompilerParams(vmem_limit_bytes=100 * 1024 * 1024),
    )(xt, A_wqkv, B_wqkv, A_wo, B_wo, gw)
    return out_t.T.reshape(1, S, D)
```

```python
import math

import jax
import jax.numpy as jnp
from jax import lax
import jax.experimental.pallas as pl
import jax.experimental.pallas.tpu as pltpu

S = 2048
D = 448
H = 16
DH = 28
HP = 32
NH = 2 * H
GW = 128
NP = NH * HP
BQ = 512
NQ = S // BQ
NT = NQ * NH
KC = 128
NC = S // KC
UN = 6
CH = 512
QSCALE = (DH ** -0.5) * math.log2(math.e)
F32 = jnp.float32
BF16 = jnp.bfloat16


def _aligned(v, m):
    return v if isinstance(v, int) else pl.multiple_of(v, m)


def _kernel(xt_hbm, wa_hbm, wb_hbm, woa_hbm, wob_hbm, gw_ref, o_hbm,
            xt_s, w_s, wo_s, wt_s, wop_s, wot_s, ktp_s, k_s, vt_s, qt_s, ot_s, sa_s, sb_s, ob_s,
            sem_w, sem_x, sem_o):
    w_cp = [pltpu.make_async_copy(src, w_s.at[b], sem_w.at[b])
            for b, src in enumerate((wa_hbm, wb_hbm))]
    wo_cp = [pltpu.make_async_copy(src, wo_s.at[b], sem_w.at[2 + b])
             for b, src in enumerate((woa_hbm, wob_hbm))]

    def x_cp(c):
        c0 = _aligned(c * CH, CH)
        return pltpu.make_async_copy(xt_hbm.at[:, pl.ds(c0, CH)], xt_s.at[:, pl.ds(c0, CH)],
                                     sem_x.at[c])

    for cp in w_cp:
        cp.start()
    for c in range(S // CH):
        x_cp(c).start()
    for cp in wo_cp:
        cp.start()

    def scatter_heads(dst, b, val, cols):
        for h in range(H):
            r0 = (b * H + h) * HP
            dst[r0:r0 + DH, cols] = val[h * DH:(h + 1) * DH, :].astype(dst.dtype)

    ktp_s[...] = jnp.zeros(ktp_s.shape, F32)
    qt_s[...] = jnp.zeros(qt_s.shape, BF16)
    rowi = lax.broadcasted_iota(jnp.int32, vt_s.shape, 0)
    vt_s[...] = jnp.where(rowi % HP == DH, 1.0, 0.0).astype(BF16)
    for b in range(2):
        w_cp[b].wait()
        wt_s[b] = w_s[b].astype(F32).T.astype(BF16)

    def proj_body(c, carry):
        c0 = pl.multiple_of(c * CH, CH)
        x_cp(c).wait()
        xc = xt_s[:, pl.ds(c0, CH)]
        for b in range(2):
            kt = jnp.dot(wt_s[b, D:2 * D, :], xc, preferred_element_type=F32)
            scatter_heads(ktp_s, b, kt, slice(None))
            vt = jnp.dot(wt_s[b, 2 * D:3 * D, :], xc, preferred_element_type=F32)
            scatter_heads(vt_s, b, vt, pl.ds(c0, CH))
            qt = jnp.dot(wt_s[b, 0:D, :], xc, preferred_element_type=F32) * QSCALE
            scatter_heads(qt_s, b, qt, pl.ds(c0, CH))
        k_s[pl.ds(c0, CH), :] = ktp_s[...].T.astype(BF16)
        return carry

    lax.fori_loop(0, S // CH, proj_body, 0)

    row = lax.broadcasted_iota(jnp.int32, (GW, BQ), 0)

    def stages(t1, s1_ref, t2, s2_ref, m2):
        if t1 is not None:
            h1 = t1 % NH
            goff = _aligned((h1 // 4) * GW, GW)
            qtg = qt_s[pl.ds(goff, GW), pl.ds(_aligned((t1 // NH) * BQ, BQ), BQ)]
            qm = jnp.where((row // HP) == (h1 % 4), qtg, jnp.zeros_like(qtg))
        if t2 is not None:
            hoff = _aligned((t2 % NH) * HP, HP)
            qoff = _aligned((t2 // NH) * BQ, BQ)
        m8 = None
        acc = None
        for c in range(NC):
            ks = slice(c * KC, (c + 1) * KC)
            if t1 is not None:
                st = jnp.dot(k_s[ks, pl.ds(goff, GW)], qm, preferred_element_type=F32)
                s1_ref[ks, :] = st
                cm = jnp.max(st.reshape(KC // 8, 8, BQ), axis=0)
                m8 = cm if m8 is None else jnp.maximum(m8, cm)
            if t2 is not None:
                pt = jnp.exp2(s2_ref[ks, :] - m2).astype(BF16)
                o = jnp.dot(vt_s[pl.ds(hoff, HP), ks], pt, preferred_element_type=F32)
                acc = o if acc is None else acc + o
        if t2 is not None:
            ot_s[pl.ds(hoff, HP), pl.ds(qoff, BQ)] = (
                acc * (1.0 / acc[DH:DH + 1, :])).astype(BF16)
        if t1 is not None:
            return jnp.max(m8, axis=0, keepdims=True)
        return None

    def loop_body(j, ma):
        for u in range(0, UN, 2):
            t = UN * j + u
            mb = stages(t + 1, sb_s, t, sa_s, ma)
            ma = stages(t + 2, sa_s, t + 1, sb_s, mb)
        return ma

    ma = stages(0, sa_s, None, None, None)
    ma = lax.fori_loop(0, (NT - 2) // UN, loop_body, ma)

    wop_s[...] = jnp.zeros(wop_s.shape, F32)
    for b in range(2):
        wo_cp[b].wait()
        scatter_heads(wop_s, b, wo_s[b].astype(F32), slice(None))
    wot_s[...] = wop_s[...].T.astype(BF16)

    mb = stages(NT - 1, sb_s, NT - 2, sa_s, ma)
    o_cp = []
    half = NP // 2

    def out_chunk(c):
        cs = slice(c * BQ, (c + 1) * BQ)
        a = jnp.dot(wot_s[:, :half], ot_s[:half, cs], preferred_element_type=F32)
        b = jnp.dot(wot_s[:, half:], ot_s[half:, cs], preferred_element_type=F32)
        gl = jnp.dot(gw_ref[...], xt_s[:, cs], preferred_element_type=F32)[0:1, :]
        gt = jax.nn.sigmoid(gl)
        ob_s[:, cs] = (gt * a + (1.0 - gt) * b).astype(BF16)
        cp = pltpu.make_async_copy(ob_s.at[:, cs], o_hbm.at[:, cs], sem_o.at[c])
        cp.start()
        o_cp.append(cp)

    out_chunk(0)
    stages(None, None, NT - 1, sb_s, mb)
    for c in range(1, NQ):
        out_chunk(c)
    for cp in o_cp:
        cp.wait()


@jax.jit
def pallas_gated_mix__mha_block__softmax_full_mha__prompt_kernel(
    A_x: jax.Array,
    A_wqkv: jax.Array,
    A_wo: jax.Array,
    B_x: jax.Array,
    B_wqkv: jax.Array,
    B_wo: jax.Array,
    gate_w: jax.Array,
):
    del B_x
    assert (NT - 2) % UN == 0 and UN % 2 == 0
    xt = A_x.reshape(S, D).T
    gw = jnp.broadcast_to(gate_w.reshape(1, D), (8, D))
    hbm = pl.BlockSpec(memory_space=pl.ANY)
    out_t = pl.pallas_call(
        _kernel,
        in_specs=[hbm, hbm, hbm, hbm, hbm, pl.BlockSpec(memory_space=pltpu.VMEM)],
        out_specs=hbm,
        out_shape=jax.ShapeDtypeStruct((D, S), BF16),
        scratch_shapes=[
            pltpu.VMEM((D, S), BF16),
            pltpu.VMEM((2, D, 3 * D), BF16),
            pltpu.VMEM((2, D, D), BF16),
            pltpu.VMEM((2, 3 * D, D), BF16),
            pltpu.VMEM((NP, D), F32),
            pltpu.VMEM((D, NP), BF16),
            pltpu.VMEM((NP, CH), F32),
            pltpu.VMEM((S, NP), BF16),
            pltpu.VMEM((NP, S), BF16),
            pltpu.VMEM((NP, S), BF16),
            pltpu.VMEM((NP, S), BF16),
            pltpu.VMEM((S, BQ), F32),
            pltpu.VMEM((S, BQ), F32),
            pltpu.VMEM((D, S), BF16),
            pltpu.SemaphoreType.DMA((4,)),
            pltpu.SemaphoreType.DMA((S // CH,)),
            pltpu.SemaphoreType.DMA((NQ,)),
        ],
        compiler_params=pltpu.CompilerParams(vmem_limit_bytes=100 * 1024 * 1024),
    )(xt, A_wqkv, B_wqkv, A_wo, B_wo, gw)
    return out_t.T.reshape(1, S, D)
```
